```python
import os as _os
_os.environ.setdefault("JAX_PLATFORMS", "cpu")
import jax
import jax.numpy as jnp

def _softmax(x, axis=-1):
    return jax.nn.softmax(x, axis=axis)
def _gelu(x):
    return jax.nn.gelu(x, approximate=True)
def _silu(x):
    return jax.nn.silu(x)
def _sigmoid(x):
    return jax.nn.sigmoid(x)
def _layernorm(x, axis=-1, eps=1e-5):
    m = jnp.mean(x, axis=axis, keepdims=True)
    v = jnp.var(x, axis=axis, keepdims=True)
    return (x - m) / jnp.sqrt(v + eps)
def _scatter_add(tgt, idx, src, axis=0):
    return tgt.at[idx].add(src)
def _segment_sum(src, seg, n):
    return jax.ops.segment_sum(src, seg, n)
class _Rng:
    def __init__(self, key):
        self._k = key
    def _next(self):
        self._k, sub = jax.random.split(self._k)
        return sub
    def normal(self, shape):
        return jax.random.normal(self._next(), shape, dtype=jnp.bfloat16)
    def randint(self, lo, hi, shape):
        return jax.random.randint(self._next(), shape, lo, hi, dtype=jnp.int32)
    def uniform(self, shape, lo=0.0, hi=1.0):
        return jax.random.uniform(self._next(), shape, jnp.bfloat16, lo, hi)
    def permutation(self, n):
        return jax.random.permutation(self._next(), n)


kernel_name = 'standalone__gqa_softmax__near_ridge'

def setup_inputs():
    _rng = _Rng(jax.random.key(int.from_bytes(__import__("os").urandom(4), "little")))
    _w = (lambda a: (lambda t: t.astype(jnp.bfloat16) if jnp.issubdtype(t.dtype, jnp.floating) else t)(jnp.asarray(a)))
    B, Hq, Hkv, Sq, Sk, D = 8, 16, 8, 512, 512, 256
    return {
        "q": _w((lambda *s: _rng.normal(s) * 0.4)(B, Hq, Sq, D)),
        "k": _w((lambda *s: _rng.normal(s) * 0.4)(B, Hkv, Sk, D)),
        "v": _w((lambda *s: _rng.normal(s) * 0.05)(B, Hkv, Sk, D)),
    }

def reference(q, k, v):
    B, Hq, Sq, D = q.shape
    Hkv = k.shape[1]
    rep = Hq // Hkv
    k = jnp.repeat(k, rep, axis=1)
    v = jnp.repeat(v, rep, axis=1)
    scale = D ** -0.5
    scores = jnp.einsum("bhqd,bhkd->bhqk", q, k) * scale
    p = _softmax(scores, axis=-1)
    return jnp.einsum("bhqk,bhkd->bhqd", p, v)
```

```python
import functools

import jax
import jax.numpy as jnp
import numpy as np
import jax.experimental.pallas as pl
import jax.experimental.pallas.tpu as pltpu

_LOG2E = float(np.log2(np.e))
_RAMP = (1, 2, 4)
_GROUP = 8
_TAIL_CHUNKS = 8


def _attention_kernel(q_hbm, k_hbm, v_hbm, o_hbm, q_buf, k_buf, vo_buf,
                      in_sems, out_sem, *, exp2_scale):
    num_heads, rows, _ = q_hbm.shape
    sk = k_hbm.shape[1]
    num_ramp = 1 + sum(_RAMP)
    num_iters = (num_heads - num_ramp) // _GROUP
    assert num_ramp + num_iters * _GROUP == num_heads

    def v_view(heads):
        return vo_buf.at[heads, pl.ds(0, sk)]

    def o_view(heads, start=0, size=rows):
        return vo_buf.at[heads, pl.ds(sk + start, size)]

    def input_copies(first_head, size, sem):
        heads = pl.ds(first_head, size)
        return [
            pltpu.make_async_copy(src, dst, in_sems.at[sem])
            for src, dst in ((k_hbm.at[heads], k_buf.at[heads]),
                             (q_hbm.at[heads], q_buf.at[heads]),
                             (v_hbm.at[heads], v_view(heads)))
        ]

    def scores(h, start=0, size=rows):
        return jax.lax.dot_general(
            q_buf[h, start:start + size, :], k_buf[h],
            (((1,), (1,)), ((), ())), preferred_element_type=jnp.float32)

    def attend(s, h):
        m = jnp.max(s, axis=-1, keepdims=True)
        p = jnp.exp2((s - m) * exp2_scale).astype(vo_buf.dtype)
        l = jnp.sum(p.astype(jnp.float32), axis=-1, keepdims=True)
        o = jnp.dot(p, v_view(h)[...], preferred_element_type=jnp.float32)
        return (o * (1.0 / l)).astype(vo_buf.dtype)

    half = rows // 2
    lo, hi = pl.ds(0, half), pl.ds(half, rows - half)
    head0_early = [
        pltpu.make_async_copy(k_hbm.at[0], k_buf.at[0], in_sems.at[0]),
        pltpu.make_async_copy(q_hbm.at[0, lo], q_buf.at[0, lo], in_sems.at[0]),
    ]
    head0_late = [
        pltpu.make_async_copy(q_hbm.at[0, hi], q_buf.at[0, hi], in_sems.at[1]),
        pltpu.make_async_copy(v_hbm.at[0], v_view(0), in_sems.at[1]),
    ]
    ramp = [(1 + sum(_RAMP[:i]), size, 2 + i) for i, size in enumerate(_RAMP)]
    loop_sem = 2 + len(_RAMP)
    for copy in head0_early + head0_late:
        copy.start()
    for group in ramp:
        for copy in input_copies(*group):
            copy.start()
    for i in range(num_iters):
        for copy in input_copies(num_ramp + i * _GROUP, _GROUP, loop_sem + i):
            copy.start()

    for copy in head0_early:
        copy.wait()
    s_lo = scores(0, 0, half)
    for copy in head0_late:
        copy.wait()
    s_hi = scores(0, half, rows - half)
    o_view(0)[...] = attend(jnp.concatenate([s_lo, s_hi], axis=0), 0)
    for first_head, size, sem in ramp:
        for copy in input_copies(first_head, size, sem):
            copy.wait()
        for h in range(first_head, first_head + size):
            o_view(h)[...] = attend(scores(h), h)

    def group_step(i, first_out):
        first_head = num_ramp + i * _GROUP

        @pl.when(i == max(num_iters - 2, 0))
        def _():
            heads = pl.ds(0, num_ramp)
            pltpu.make_async_copy(o_view(heads), o_hbm.at[heads], out_sem).start()

        for copy in input_copies(first_head, _GROUP, loop_sem + i):
            copy.wait()
        for g in range(_GROUP):
            o = attend(scores(first_head + g), first_head + g)
            size = rows // (_TAIL_CHUNKS if g == _GROUP - 1 else 1)
            for start in range(0, rows, size):
                chunk = o_view(first_out + g, start, size)
                chunk[...] = o[start:start + size]
                pltpu.make_async_copy(
                    chunk, o_hbm.at[first_out + g, pl.ds(start, size)],
                    out_sem).start()
        return first_out + _GROUP

    jax.lax.fori_loop(0, num_iters, group_step, np.int32(num_ramp))
    pltpu.make_async_copy(o_view(pl.ds(0, num_heads)), o_hbm, out_sem).wait()


@jax.jit
def pallas_standalone__gqa_softmax__near_ridge_kernel(
    q: jax.Array,
    k: jax.Array,
    v: jax.Array,
):
    B, Hq, Sq, D = q.shape
    _, Hkv, Sk, _ = k.shape
    num_heads = B * Hkv
    rows = (Hq // Hkv) * Sq
    num_groups = 2 + len(_RAMP) + (num_heads - 1 - sum(_RAMP)) // _GROUP

    out = pl.pallas_call(
        functools.partial(_attention_kernel, exp2_scale=D ** -0.5 * _LOG2E),
        in_specs=[pl.BlockSpec(memory_space=pl.ANY)] * 3,
        out_specs=pl.BlockSpec(memory_space=pl.ANY),
        out_shape=jax.ShapeDtypeStruct((num_heads, rows, D), q.dtype),
        scratch_shapes=[
            pltpu.VMEM((num_heads, rows, D), q.dtype),
            pltpu.VMEM((num_heads, Sk, D), k.dtype),
            pltpu.VMEM((num_heads, Sk + rows, D), v.dtype),
            pltpu.SemaphoreType.DMA((num_groups,)),
            pltpu.SemaphoreType.DMA(()),
        ],
        compiler_params=pltpu.CompilerParams(
            vmem_limit_bytes=116 * 1024 * 1024,
        ),
    )(
        q.reshape(num_heads, rows, D),
        k.reshape(num_heads, Sk, D),
        v.reshape(num_heads, Sk, D),
    )
    return out.reshape(B, Hq, Sq, D)
```

```python
import functools

import jax
import jax.numpy as jnp
import numpy as np
import jax.experimental.pallas as pl
import jax.experimental.pallas.tpu as pltpu

_LOG2E = float(np.log2(np.e))
_GROUP = 16
_LOOKAHEAD = 2
_LEAD_CHUNKS = 4
_TAIL_CHUNKS = 16


def _attention_kernel(q_hbm, k_hbm, v_hbm, o_hbm, buf, in_sems, out_sem, *,
                      exp2_scale):
    num_heads, rows, _ = q_hbm.shape
    sk = k_hbm.shape[1]
    num_groups = num_heads // _GROUP
    assert num_heads % _GROUP == 0 and _GROUP % _LOOKAHEAD == 0

    def k_view(h):
        return buf.at[h, pl.ds(0, sk)]

    def v_view(h):
        return buf.at[h, pl.ds(sk, sk)]

    def q_view(h, start, size):
        return buf.at[h, pl.ds(2 * sk + start, size)]

    def o_view(h, start, size):
        return buf.at[h, pl.ds(2 * sk + rows + start, size)]

    def row_chunks(count):
        return [(c * (rows // count), rows // count) for c in range(count)]

    def q_chunks(g):
        return row_chunks(_LEAD_CHUNKS if g == 0 else 1)

    def kq_copies(h, g, chunk=0):
        start, size = q_chunks(g)[chunk]
        q_src, q_dst = q_hbm.at[h, pl.ds(start, size)], q_view(h, start, size)
        if chunk > 0:
            sem = in_sems.at[2 * _LOOKAHEAD + chunk - 1]
            return [pltpu.make_async_copy(q_src, q_dst, sem)]
        sem = in_sems.at[2 * (g % _LOOKAHEAD)]
        return [pltpu.make_async_copy(k_hbm.at[h], k_view(h), sem),
                pltpu.make_async_copy(q_src, q_dst, sem)]

    def v_copy(h, g):
        sem = in_sems.at[2 * (g % _LOOKAHEAD) + 1]
        return pltpu.make_async_copy(v_hbm.at[h], v_view(h), sem)

    def start_inputs(h, g):
        for chunk in range(len(q_chunks(g))):
            for copy in kq_copies(h, g, chunk):
                copy.start()
        v_copy(h, g).start()

    def attend(i, g):
        h = i * _GROUP + g

        s = []
        for chunk, (start, size) in enumerate(q_chunks(g)):
            if g == 0:
                for copy in kq_copies(h, g, chunk):
                    copy.wait()
            s.append(jax.lax.dot_general(
                q_view(h, start, size)[...], k_view(h)[...],
                (((1,), (1,)), ((), ())), preferred_element_type=jnp.float32))
        s = jnp.concatenate(s, axis=0) if len(s) > 1 else s[0]

        v_copy(h, g).wait()
        prefetch = functools.partial(
            start_inputs, h + _LOOKAHEAD, (g + _LOOKAHEAD) % _GROUP)
        if g + _LOOKAHEAD < _GROUP:
            prefetch()
        else:
            pl.when(i + 1 < num_groups)(prefetch)

        m = jnp.max(s, axis=-1, keepdims=True)
        p = jnp.exp2((s - m) * exp2_scale).astype(buf.dtype)
        l = jnp.sum(p.astype(jnp.float32), axis=-1, keepdims=True)
        o = jnp.dot(p, v_view(h)[...], preferred_element_type=jnp.float32)
        o = (o * pltpu.reciprocal(l, full_range=False)).astype(buf.dtype)

        if g + 1 < _GROUP:
            for copy in kq_copies(h + 1, g + 1):
                copy.wait()

        for start, size in row_chunks(_TAIL_CHUNKS if g + 1 == _GROUP else 1):
            o_view(h, start, size)[...] = o[start:start + size]
            pltpu.make_async_copy(
                o_view(h, start, size), o_hbm.at[h, pl.ds(start, size)],
                out_sem).start()

    def group_step(i, carry):
        for g in range(_GROUP):
            attend(i, g)
        return carry

    for g in range(_LOOKAHEAD):
        start_inputs(g, g)
    jax.lax.fori_loop(0, num_groups, group_step, None)
    pltpu.make_async_copy(
        o_view(pl.ds(0, num_heads), 0, rows), o_hbm, out_sem).wait()


@jax.jit
def pallas_standalone__gqa_softmax__near_ridge_kernel(
    q: jax.Array,
    k: jax.Array,
    v: jax.Array,
):
    B, Hq, Sq, D = q.shape
    _, Hkv, Sk, _ = k.shape
    num_heads = B * Hkv
    rows = (Hq // Hkv) * Sq

    out = pl.pallas_call(
        functools.partial(_attention_kernel, exp2_scale=D ** -0.5 * _LOG2E),
        in_specs=[pl.BlockSpec(memory_space=pl.ANY)] * 3,
        out_specs=pl.BlockSpec(memory_space=pl.ANY),
        out_shape=jax.ShapeDtypeStruct((num_heads, rows, D), q.dtype),
        scratch_shapes=[
            pltpu.VMEM((num_heads, 2 * Sk + 2 * rows, D), q.dtype),
            pltpu.SemaphoreType.DMA((2 * _LOOKAHEAD + _LEAD_CHUNKS - 1,)),
            pltpu.SemaphoreType.DMA(()),
        ],
        compiler_params=pltpu.CompilerParams(
            vmem_limit_bytes=116 * 1024 * 1024,
            disable_bounds_checks=True,
            flags={"XLA_TPU_RESCHEDULE_DMA_DONES": True},
        ),
    )(
        q.reshape(num_heads, rows, D),
        k.reshape(num_heads, Sk, D),
        v.reshape(num_heads, Sk, D),
    )
    return out.reshape(B, Hq, Sq, D)
```
